```python
import os as _os
_os.environ.setdefault("JAX_PLATFORMS", "cpu")
import jax
import jax.numpy as jnp

def _softmax(x, axis=-1):
    return jax.nn.softmax(x, axis=axis)
def _gelu(x):
    return jax.nn.gelu(x, approximate=True)
def _silu(x):
    return jax.nn.silu(x)
def _sigmoid(x):
    return jax.nn.sigmoid(x)
def _layernorm(x, axis=-1, eps=1e-5):
    m = jnp.mean(x, axis=axis, keepdims=True)
    v = jnp.var(x, axis=axis, keepdims=True)
    return (x - m) / jnp.sqrt(v + eps)
def _scatter_add(tgt, idx, src, axis=0):
    return tgt.at[idx].add(src)
def _segment_sum(src, seg, n):
    return jax.ops.segment_sum(src, seg, n)
class _Rng:
    def __init__(self, key):
        self._k = key
    def _next(self):
        self._k, sub = jax.random.split(self._k)
        return sub
    def normal(self, shape):
        return jax.random.normal(self._next(), shape, dtype=jnp.bfloat16)
    def randint(self, lo, hi, shape):
        return jax.random.randint(self._next(), shape, lo, hi, dtype=jnp.int32)
    def uniform(self, shape, lo=0.0, hi=1.0):
        return jax.random.uniform(self._next(), shape, jnp.bfloat16, lo, hi)
    def permutation(self, n):
        return jax.random.permutation(self._next(), n)


kernel_name = 'gated_mix__spectral_gfnet__dense_activation_silu__prompt'

def setup_inputs():
    _rng = _Rng(jax.random.key(int.from_bytes(__import__("os").urandom(4), "little")))
    _w = (lambda a: (lambda t: t.astype(jnp.bfloat16) if jnp.issubdtype(t.dtype, jnp.floating) else t)(jnp.asarray(a)))
    def _A_setup():
        B, S, D = 1, 2048, 512
        Df = D // 2 + 1
        return {
            "x": _w((lambda *s: _rng.normal(s) * 0.05)(B, S, D)),
            "w_r": _w((lambda *s: _rng.normal(s) * 0.05)(S, Df) * 0.02),
            "w_i": _w((lambda *s: _rng.normal(s) * 0.05)(S, Df) * 0.02),
        }
    _A_in = _A_setup()

    def _B_setup():
        B, S, D, F = 1, 2048, 512, 1376
        return {
            "x": _w((lambda *s: _rng.normal(s) * 0.05)(B, S, D)),
            "w1": _w((lambda *s: _rng.normal(s) * 0.05)(D, F) * (D ** -0.5)),
            "w2": _w((lambda *s: _rng.normal(s) * 0.05)(F, D) * (F ** -0.5)),
        }
    _B_in = _B_setup()

    return {
        "A_x": _A_in["x"],
        "A_w_r": _A_in["w_r"],
        "A_w_i": _A_in["w_i"],
        "B_x": _B_in["x"],
        "B_w1": _B_in["w1"],
        "B_w2": _B_in["w2"],
        "gate_w": _w((lambda *s: _rng.normal(s) * 0.05)(512) * 16.0),
    }

def reference(A_x, A_w_r, A_w_i, B_x, B_w1, B_w2, gate_w):
    def _A_ref(x, w_r, w_i):
        B, S, D = x.shape
        X = (lambda x, axes=(-2,-1): jnp.fft.rfft2(x.astype(jnp.float32), axes=axes))(x, axes=(-2, -1))
        W = w_r + 1j * w_i
        X = X * W
        y = (lambda x, s, axes=(-2,-1): jnp.fft.irfft2(x, s=s, axes=axes).astype(jnp.bfloat16))(X, (S, D), axes=(-2, -1))
        return y

    def _B_ref(x, w1, w2):
        h = jnp.einsum("bsd,df->bsf", x, w1)
        h = _silu(h)
        out = jnp.einsum("bsf,fd->bsd", h, w2)
        return out

    x = A_x
    g = _sigmoid((x * gate_w).sum(-1, keepdims=True))
    a = _A_ref(x, A_w_r, A_w_i)
    b = _B_ref(x, B_w1, B_w2)
    return g * a + (1 - g) * b
```

```python
import numpy as np
import jax
import jax.numpy as jnp
from jax import lax
import jax.experimental.pallas as pl
import jax.experimental.pallas.tpu as pltpu

S, D, F = 2048, 512, 1376
R, L = 16, 128
RB = 256
NB = S // RB
BF = jnp.bfloat16
F32 = jnp.float32
def _tw(vr, vi, num, den, sign):
    num %= den
    if num == 0: return vr, vi
    if 4 * num == den: return (-vi, vr) if sign > 0 else (vi, -vr)
    if 2 * num == den: return -vr, -vi
    if 4 * num == 3 * den: return (vi, -vr) if sign > 0 else (-vi, vr)
    c = float(np.cos(2 * np.pi * num / den)); s = float(sign * np.sin(2 * np.pi * num / den))
    if abs(abs(c) - abs(s)) < 1e-9:
        if c * s > 0: return (vr - vi) * c, (vr + vi) * c
        return (vr + vi) * c, (vi - vr) * c
    return vr * c - vi * s, vr * s + vi * c


def _dft4(x, sign):
    (ar, ai), (br, bi), (cr, ci), (dr, di) = x
    t0r, t0i = ar + cr, ai + ci
    t1r, t1i = ar - cr, ai - ci
    t2r, t2i = br + dr, bi + di
    t3r, t3i = br - dr, bi - di
    if sign < 0:
        o1 = (t1r + t3i, t1i - t3r); o3 = (t1r - t3i, t1i + t3r)
    else:
        o1 = (t1r - t3i, t1i + t3r); o3 = (t1r + t3i, t1i - t3r)
    return [(t0r + t2r, t0i + t2i), o1, (t0r - t2r, t0i - t2i), o3]


def _dft16(x, sign):
    st = [_dft4([x[4 * a + b] for a in range(4)], sign) for b in range(4)]
    out = [None] * 16
    for p in range(4):
        y = _dft4([_tw(*st[b][p], b * p, 16, sign) for b in range(4)], sign)
        for q in range(4): out[p + 4 * q] = y[q]
    return out


def _consts():
    n = np.arange(D)[None, :].astype(np.float64)
    def rows(g):
        k = (4 * np.arange(64) + g)[:, None]
        ang = 2 * np.pi * k * n / D
        return np.cos(ang), -np.sin(ang)
    c0, s0 = rows(0); c1, s1 = rows(1); c2, s2 = rows(2); c3, s3 = rows(3)
    alt = np.zeros((16, 128)); alt[0] = (-1.0) ** np.arange(128)
    f0 = np.concatenate([c0[:, :128], s0[:, :128], alt])
    f2 = np.concatenate([c2[:, :128], s2[:, :128]])
    fo = np.concatenate([c1[:, :256], c3[:, :256], s1[:, :256], s3[:, :256]])
    g0 = 2 * f0[:128].T.copy(); g0[:, 0] *= 0.5
    g2 = 2 * f2.T; go = 2 * fo.T
    ms = []
    for j in range(R):
        l = np.arange(L)[:, None]; kk = np.arange(L)[None, :]
        a = 2 * np.pi * (((R * l + j) * kk) % S) / S
        c, s = np.cos(a), np.sin(a)
        ms.append(np.block([[c, -s], [s, c]]))
    ms = np.stack(ms)
    mi = np.transpose(ms, (0, 2, 1)) / S
    import ml_dtypes
    t = lambda a: np.asarray(a, np.float32).astype(ml_dtypes.bfloat16)
    fa = np.zeros((3, 256, 256)); fa[0] = fo; fa[1, :144, :128] = f0; fa[1, :128, 128:] = f2
    fa[2] = go / D
    ga = np.concatenate([g0, g2], 1) / D
    return t(fa), t(ga), t(ms), t(mi)


NT = (((1,), (1,)), ((), ()))
KR = 272


def _mo(a, b):
    return a if isinstance(a, int) else pl.multiple_of(a, b)


def _half(w, odd):
    return pltpu.bitcast((w & jnp.uint32(0xFFFF0000)) if odd else (w << 16), F32)


def _kernel(x_h, wr_h, wi_h, w1_h, w2_h, gw_ref, f_h, g_h, m_h, mi_h, o_h,
            x_v, o_v, xn_v, p_v, w1_v, w2_v, wr_v, wi_v, f_v, g_v, m_v, mi_v, v_v, y_v, b_v, wl_v, sems, wsem, osem, fsem):
    E = [0, 128, 384, 640, 896, 1152, F]
    cp = pltpu.make_async_copy
    cx = [cp(x_h.at[0, pl.ds(i * RB, RB)], xn_v.at[pl.ds(i * RB, RB)], osem.at[i]) for i in range(NB)]
    c1 = [cp(w1_h.at[a:b], w1_v.at[a:b], fsem.at[0, k]) for k, (a, b) in enumerate(zip(E, E[1:]))]
    c2 = [cp(w2_h.at[a:b], w2_v.at[a:b], fsem.at[1, k]) for k, (a, b) in enumerate(zip(E, E[1:]))]
    cs = [cp(f_h, f_v, sems.at[0]), cp(m_h, m_v, sems.at[1])] + [cp(x_h.at[0, :, pl.ds(t * 128, 128)], x_v.at[t].bitcast(BF), sems.at[2 + t]) for t in range(4)]
    cl = [cp(mi_h, mi_v, sems.at[6]), cp(g_h, g_v, sems.at[7])]
    cw = []
    for src, dst in ((wr_h, wr_v), (wi_h, wi_v)):
        for r in range(R):
            cw.append(cp(src.at[pl.ds(0, 256), pl.ds(r * 128, 128)], dst.at[r].bitcast(BF), wsem))
    cw += [cp(wr_h.at[pl.ds(248, 9)], wl_v.at[0], wsem), cp(wi_h.at[pl.ds(248, 9)], wl_v.at[1], wsem)]
    cx[0].start(); c1[0].start(); c2[0].start(); c1[1].start(); c2[1].start()
    gw = gw_ref[...].astype(F32).reshape(1, D)

    def p1(q, _):
        xw = [x_v[t, pl.ds(q, L, stride=8), :] for t in range(4)]
        xs = [jnp.concatenate([_half(w, 0), _half(w, 1)], 0) for w in xw]
        e0, e1 = xs[0] + xs[2], xs[1] + xs[3]
        cd = jnp.concatenate([xs[0] - xs[2], xs[1] - xs[3]], 1).astype(BF)
        z0 = lax.dot_general(f_v[1, :144, :128], (e0 + e1).astype(BF), NT, preferred_element_type=F32)
        z2 = lax.dot_general(f_v[1, :128, 128:], (e0 - e1).astype(BF), NT, preferred_element_type=F32)
        zo = lax.dot_general(f_v[0], cd, NT, preferred_element_type=F32)
        zr = jnp.concatenate([z0[:64], z2[:64], zo[:128], z0[128:]], 0).astype(BF)
        zi = jnp.concatenate([z0[64:128], z2[64:], zo[128:], jnp.zeros((16, 256), F32)], 0).astype(BF)
        for o in range(2):
            z = jnp.concatenate([zr[:, o * 128:o * 128 + 128], zi[:, o * 128:o * 128 + 128]], 1)
            v_v[2 * q + o] = jnp.dot(z, m_v[2 * q + o], preferred_element_type=F32)
        return _
    def ffn(r0, work=(), first=False):
        xb = xn_v[pl.ds(r0, RB), :]
        edges = E if not work else list(range(0, 1281, 128)) + [F]
        acc = pend = None
        for k, (f0, f1) in enumerate(zip(edges, edges[1:])):
            if first:
                if k + 2 < 6: c1[k + 2].start(); c2[k + 2].start()
                if k == 3: cx[1].start(); cx[2].start()
                if k == 4:
                    for c in cs: c.start()
                c1[k].wait(); c2[k].wait()
            h = lax.dot_general(xb, w1_v[f0:f1, :], NT, preferred_element_type=F32) * 0.5
            dep = h[:8, :128] if f1 < F else dep
            h = (h * jnp.tanh(h) + h).astype(BF)
            if pend is not None:
                o = jnp.dot(pend[0], w2_v[pend[1]:pend[2], :], preferred_element_type=F32)
                acc = o if acc is None else acc + o
            pend = (h, f0, f1)
            for _ in range(1 + (0) if work is allw else 1):
                if work: work.pop(0)(dep)
        return acc + jnp.dot(pend[0], w2_v[pend[1]:pend[2], :], preferred_element_type=F32)

    def mid(k0, wload, dep):
        xs = [(v_v[j, pl.ds(k0, 8), :128], v_v[j, pl.ds(k0, 8), 128:]) for j in range(R)]
        keep = f_v[1, 208:224, 128:].astype(F32)[:8] == 0.0
        xs = [(jnp.where(keep, a, dep), jnp.where(keep, b, dep)) for a, b in xs]
        xs = _dft16(xs, -1)
        ys = []
        for r in range(R):
            a, b = wload(wr_v, r), wload(wi_v, r)
            zr, zi = xs[r]
            ys.append((zr * a - zi * b, zr * b + zi * a))
        ys = _dft16(ys, +1)
        for j in range(R):
            p_v[j, pl.ds(k0, 8), :128] = ys[j][0]
            p_v[j, pl.ds(k0, 8), 128:] = ys[j][1]

    allw = []

    def p2(i, _):
        hi = i // 2
        work = allw
        for u in range(4):
            for odd in range(2):
                a = (i % 2) * 4 + u
                work.append(lambda dep, a=a, odd=odd, hi=hi: mid(_mo(odd * 128 + hi * 64 + a * 8, 8),
                            lambda ref, r: _half(ref[r, pl.ds(a * 16 + hi, 8, stride=2), :], odd), dep))
        return _
    cx[0].wait()
    b_v[0:RB, :] = ffn(0, first=True)
    for c in cx[3:5] + cw + cl + cx[5:]: c.start()

    def fblk(i, work=()):
        r0 = _mo(i * RB, RB)
        b_v[pl.ds(r0, RB), :] = ffn(r0, work)

    def pa(i, _):
        cp(x_h.at[0, pl.ds(0, RB)], xn_v.at[pl.ds(0, RB)], osem.at[i]).wait()
        fblk(i)
        return _
    lax.fori_loop(1, 3, pa, None)
    for c in cs: c.wait()
    lax.fori_loop(0, 2, lambda q, _: [p1(4 * q + t, _) for t in range(4)][0], None)
    for c in cx[3:] + cw: c.wait()

    def pb(i, _):
        p2(i, None)
        fblk(i + 3, allw)
        return _
    for q in range(4): p2(q, None)
    for i in (3, 4, 5): fblk(i, allw)
    row0 = lax.broadcasted_iota(jnp.int32, (8, 128), 0) == 0
    mid(256, lambda ref, r: jnp.where(row0, wl_v[0 if ref is wr_v else 1, 8:9, r * 128:(r + 1) * 128].astype(F32), 0.0), jnp.zeros((8, 128), F32))
    for c in cl: c.wait()

    def p3(q, _):
        sgn = (1 - 2 * (lax.broadcasted_iota(jnp.int32, (L, 256), 0) & 1)).astype(F32) * (1.0 / D)
        ts = [jnp.dot(jnp.concatenate([p_v[j, :264], jnp.zeros((8, 256), F32)], 0).astype(BF), mi_v[j], preferred_element_type=F32)
              for j in (2 * q, 2 * q + 1)]
        tb = [t[:256].astype(BF) for t in ts]
        rhs = lambda a, b: jnp.concatenate([jnp.concatenate([t[a:b, :128], t[a:b, 128:]], 0) for t in tb], 1)
        p0 = jnp.dot(g_v[:, :128], rhs(0, 64), preferred_element_type=F32)
        p2_ = jnp.dot(g_v[:, 128:], rhs(64, 128), preferred_element_type=F32)
        po = jnp.dot(f_v[2], rhs(128, 256), preferred_element_type=F32)
        p0 = p0 + sgn * jnp.concatenate([t[256:257, :128] for t in ts], 1)
        s, d = p0 + p2_, p0 - p2_
        ys = [s + po[:128], d + po[128:], s - po[:128], d - po[128:]]
        ys = [pltpu.bitcast(v.astype(BF).astype(F32), jnp.uint32) for v in ys]
        outs = [[v[:, :128] for v in ys], [v[:, 128:] for v in ys]]
        for tt in range(4):
            y_v[tt, pl.ds(q, L, stride=8), :] = ((outs[0][tt] >> 16) | outs[1][tt]).T
        return _
    lax.fori_loop(0, 2, lambda q, _: [p3(4 * q + t, _) for t in range(4)][0], None)

    def emit(i, b):
        r0 = _mo(i * RB, RB)
        xb = xn_v[pl.ds(r0, RB), :].astype(F32)
        pr = xb * gw
        g = 0.5 + 0.5 * jnp.tanh(0.5 * jnp.sum(pr, axis=-1, keepdims=True))
        y = jnp.concatenate([pltpu.bitcast(y_v[t, pl.ds(r0 // 2, RB // 2), :], BF) for t in range(4)], 1).astype(F32)
        o_v[pl.ds(r0, RB), :] = (b + g * (y - b)).astype(BF)
        pltpu.make_async_copy(o_v.at[pl.ds(r0, RB)], o_h.at[0, pl.ds(r0, RB)], osem.at[i]).start()

    emit(6, ffn(6 * RB, [lambda dep, i=i: emit(i, b_v[pl.ds(i * RB, RB), :]) for i in range(6)]))
    emit(7, ffn(7 * RB))
    for i in range(NB):
        pltpu.make_async_copy(o_v.at[pl.ds(i * RB, RB)], o_h.at[0, pl.ds(i * RB, RB)], osem.at[i]).wait()


@jax.jit
def pallas_gated_mix__spectral_gfnet__dense_activation_silu__prompt_kernel(A_x, A_w_r, A_w_i, B_x, B_w1, B_w2, gate_w):
    fa, ga, ms, mi = _consts()
    hbm = pl.BlockSpec(memory_space=pltpu.HBM)
    V = pltpu.VMEM
    return pl.pallas_call(
        _kernel,
        out_shape=jax.ShapeDtypeStruct((1, S, D), BF),
        in_specs=[hbm] * 5 + [pl.BlockSpec(memory_space=V)] + [hbm] * 4,
        out_specs=hbm,
        scratch_shapes=[V((4, S // 2, 128), jnp.uint32), V((S, D), BF), V((S, D), BF), V((R, KR, 256), F32), V((F, D), BF), V((F, D), BF), V((R, 128, 128), jnp.uint32), V((R, 128, 128), jnp.uint32),
                        V((3, 256, 256), BF), V((128, 256), BF), V((R, 256, 256), BF), V((R, 256, 256), BF),
                        V((R, KR, 256), F32), V((4, S // 2, 128), jnp.uint32), V((7 * RB, D), F32), V((2, 9, S), BF),
                        pltpu.SemaphoreType.DMA((11,)), pltpu.SemaphoreType.DMA(()), pltpu.SemaphoreType.DMA((NB,)), pltpu.SemaphoreType.DMA((2, 6))],
        compiler_params=pltpu.CompilerParams(vmem_limit_bytes=100 * 1024 * 1024),
    )(A_x, A_w_r.T, A_w_i.T, B_w1.T, B_w2, gate_w, fa, ga, ms, mi)
```
